```python
import os as _os
_os.environ.setdefault("JAX_PLATFORMS", "cpu")
import jax
import jax.numpy as jnp

def _softmax(x, axis=-1):
    return jax.nn.softmax(x, axis=axis)
def _gelu(x):
    return jax.nn.gelu(x, approximate=True)
def _silu(x):
    return jax.nn.silu(x)
def _sigmoid(x):
    return jax.nn.sigmoid(x)
def _layernorm(x, axis=-1, eps=1e-5):
    m = jnp.mean(x, axis=axis, keepdims=True)
    v = jnp.var(x, axis=axis, keepdims=True)
    return (x - m) / jnp.sqrt(v + eps)
def _scatter_add(tgt, idx, src, axis=0):
    return tgt.at[idx].add(src)
def _segment_sum(src, seg, n):
    return jax.ops.segment_sum(src, seg, n)
class _Rng:
    def __init__(self, key):
        self._k = key
    def _next(self):
        self._k, sub = jax.random.split(self._k)
        return sub
    def normal(self, shape):
        return jax.random.normal(self._next(), shape, dtype=jnp.bfloat16)
    def randint(self, lo, hi, shape):
        return jax.random.randint(self._next(), shape, lo, hi, dtype=jnp.int32)
    def uniform(self, shape, lo=0.0, hi=1.0):
        return jax.random.uniform(self._next(), shape, jnp.bfloat16, lo, hi)
    def permutation(self, n):
        return jax.random.permutation(self._next(), n)


kernel_name = 'standalone__softmax_full_bidir__sampling'

def setup_inputs():
    _rng = _Rng(jax.random.key(int.from_bytes(__import__("os").urandom(4), "little")))
    _w = (lambda a: (lambda t: t.astype(jnp.bfloat16) if jnp.issubdtype(t.dtype, jnp.floating) else t)(jnp.asarray(a)))
    B, H, Sq, Skv, Dh = 8, 32, 1, 4096, 192
    return {
        "q": _w((lambda *s: _rng.normal(s) * 0.4)(B, H, Sq, Dh)),
        "k": _w((lambda *s: _rng.normal(s) * 0.4)(B, H, Skv, Dh)),
        "v": _w((lambda *s: _rng.normal(s) * 0.05)(B, H, Skv, Dh)),
    }

def reference(q, k, v):
    scale = q.shape[-1] ** -0.5
    scores = jnp.einsum('bhqd,bhkd->bhqk', q, k) * scale
    attn = _softmax(scores, axis=-1)
    return jnp.einsum('bhqk,bhkd->bhqd', attn, v)
```

```python
import functools
import jax, jax.numpy as jnp, numpy as np
from jax import lax
from jax.experimental import pallas as pl
from jax.experimental.pallas import tpu as pltpu

def make_v2(NH=4, sub=1, nslot=3, compute=True, bursts=None):
    def fn(q, k, v):
        B, H, Sq, Dh = q.shape
        Skv = k.shape[2]
        G = B * H
        scale = Dh ** -0.5
        q2 = q.reshape(G, Dh)
        kT = jnp.swapaxes(k, 2, 3).reshape(G, Dh, Skv)
        vT = jnp.swapaxes(v, 2, 3).reshape(G, Dh, Skv)
        RB = 16
        NG = G // NH
        R = Dh // sub
        PC = 2048
        pcs = [(h, s * R + r, c) for r in range(0, R, 8) for c in range(0, Skv, PC) for h in range(NH) for s in range(sub)]
        npc = len(pcs)
        def kernel(q_hbm, k_hbm, v_hbm, o_hbm, q_ref, o_ref, kbuf, vbuf, acc_ref, sem, sem2):
            def issue(g, slot, lo, hi):
                for (h, r, c) in pcs[lo:hi]:
                    pltpu.make_async_copy(k_hbm.at[g * NH + h, pl.ds(r, 8), pl.ds(c, PC)], kbuf.at[slot, h, pl.ds(r, 8), pl.ds(c, PC)], sem.at[0, slot]).start(priority=0)
                    pltpu.make_async_copy(v_hbm.at[g * NH + h, pl.ds(r, 8), pl.ds(c, PC)], vbuf.at[slot, h, pl.ds(r, 8), pl.ds(c, PC)], sem.at[1, slot]).start(priority=1)
            def wait(slot):
                pltpu.make_async_copy(kbuf.at[slot], kbuf.at[slot], sem.at[0, slot]).wait()
                pltpu.make_async_copy(vbuf.at[slot], vbuf.at[slot], sem.at[1, slot]).wait()
            def head(g, slot, j):
                if not compute: return
                hh = g * NH + j
                rb = pl.multiple_of(hh // RB * RB, RB)
                qb = q_ref[pl.ds(rb, RB), :]
                s = jnp.dot(qb, kbuf[slot, j], preferred_element_type=jnp.float32) * scale
                m = jnp.max(s, axis=-1, keepdims=True)
                p = jnp.exp(s - m)
                l = jnp.sum(p, axis=-1, keepdims=True)
                o = lax.dot_general(p.astype(jnp.bfloat16), vbuf[slot, j], (((1,), (1,)), ((), ())), preferred_element_type=jnp.float32)
                o = o / l
                row = lax.broadcasted_iota(jnp.int32, (RB, Dh), 0)
                a = jnp.where(row == hh % RB, o, acc_ref[...])
                acc_ref[...] = a
                o_ref[pl.ds(rb, RB), :] = a.astype(o_ref.dtype)
            qc = pltpu.make_async_copy(q_hbm, q_ref, sem2.at[0])
            qc.start()
            acc_ref[...] = jnp.zeros_like(acc_ref)
            if not compute: o_ref[...] = jnp.zeros_like(o_ref)
            LA = nslot - 1
            for g in range(LA):
                issue(g, g, 0, npc)
            qc.wait()
            def body(g, slot):
                nslot_i = jnp.where(slot == 0, nslot - 1, slot - 1)
                wait(slot)
                for j in range(NH):
                    issue(g + LA, nslot_i, j * npc // NH, (j + 1) * npc // NH)
                    head(g, slot, j)
                return jnp.where(slot == nslot - 1, 0, slot + 1)
            lax.fori_loop(0, NG - LA, body, jnp.int32(0))
            for g in range(NG - LA, NG):
                wait(g % nslot)
                lax.fori_loop(0, NH, lambda j, _: head(g, g % nslot, j), None)
            oc = pltpu.make_async_copy(o_ref, o_hbm, sem2.at[1])
            oc.start(); oc.wait()
        anyspec = pl.BlockSpec(memory_space=pl.ANY)
        out = pl.pallas_call(
            kernel,
            in_specs=[anyspec] * 3,
            out_specs=anyspec,
            out_shape=jax.ShapeDtypeStruct((G, Dh), q.dtype),
            scratch_shapes=[pltpu.VMEM((G, Dh), q.dtype), pltpu.VMEM((G, Dh), q.dtype),
                            pltpu.VMEM((nslot, NH, Dh, Skv), k.dtype), pltpu.VMEM((nslot, NH, Dh, Skv), v.dtype),
                            pltpu.VMEM((RB, Dh), jnp.float32),
                            pltpu.SemaphoreType.DMA((2, nslot)), pltpu.SemaphoreType.DMA((2,))],
            compiler_params=pltpu.CompilerParams(vmem_limit_bytes=120 * 1024 * 1024, disable_bounds_checks=True),
        )(q2, kT, vT)
        return out.reshape(B, H, Sq, Dh)
    return fn


@jax.jit
def pallas_standalone__softmax_full_bidir__sampling_kernel(q, k, v):
    return make_v2(2, 2, 3, True)(q, k, v)
```

```python
import functools

import jax
import jax.numpy as jnp
from jax import lax
import jax.experimental.pallas as pl
import jax.experimental.pallas.tpu as pltpu

_PARTS = 3
_BATCHES = 4
_ROWS = 8
_LAG = 26
_IN_FLIGHT = 32
_SLOTS = 4
_WAIT_BURST = 5
_LAST_STEP = (
    ((0, 0, 4), (1, 0, 4)),
    ((2, 0, 4), (3, 0, 4)),
    ((0, 4, 4), (1, 4, 4)),
    ((2, 4, 2), (3, 4, 2)),
    ((2, 6, 2),),
    ((3, 6, 1),),
    ((3, 7, 1),),
)


def _aligned(x, n):
  return x if isinstance(x, int) else pl.multiple_of(x, n)


def _kernel(q_hbm, k_hbm, v_hbm, o_hbm,
            q_ref, q_parts, buf, s_ref, p_ref, rl_ref, acc_ref, o_ref,
            step_sem, last_sem, io_sem, *, heads, scale):
  n_heads, dh = q_hbm.shape
  skv = k_hbm.shape[1]
  chunk = dh // _PARTS
  streams = _PARTS * _BATCHES
  groups = n_heads // (heads * _BATCHES)
  steps = groups * heads
  burst_rows = chunk // _BATCHES
  half = skv // 2
  pairs = [(r, c, m) for r in range(0, burst_rows, _ROWS) for c in (0, half)
           for m in range(0, streams, 2)]
  first_v = steps * _BATCHES
  first_last = (2 * steps - 1) * _BATCHES
  early = pl.cdiv(_LAG, len(pairs))

  def div(x, n):
    return x // n if isinstance(x, int) else lax.div(x, n)

  def rem(x, n):
    return x % n if isinstance(x, int) else lax.rem(x, n)

  def locate(step):
    return rem(div(step, heads), groups), rem(step, heads), rem(step, _SLOTS)

  def copier(src, step, sem=None):
    group, u, slot = locate(step)
    base = (group * streams * heads + u) * chunk
    part = [rem(j * heads + u, _PARTS) * chunk for j in range(_PARTS)]

    def copy(m, r, rows, c, cols, sem):
      batch, j = divmod(m, _PARTS)
      return pltpu.make_async_copy(
          src.at[pl.ds(_aligned(base + m * heads * chunk + r, _ROWS), rows),
                 pl.ds(c, cols)],
          buf.at[slot, batch, pl.ds(_aligned(part[j] + r, _ROWS), rows),
                 pl.ds(c, cols)],
          step_sem.at[slot] if sem is None else sem)

    return copy

  last_copy = copier(v_hbm, 2 * steps - 1)
  last = []
  for i, blocks in enumerate(_LAST_STEP):
    pieces = []
    for batch, c, w in blocks:
      rows = min(chunk, 4 * _ROWS // w)
      pieces += [(r, _PARTS * batch + j, rows, c * skv // 8, w * skv // 8)
                 for r in range(0, chunk, rows) for j in range(_PARTS)]
    last += [(i, last_copy(m, r, rows, c, w, last_sem.at[i]))
             for r, m, rows, c, w in sorted(pieces)]
  paired = len(last) - _LAG
  last_by_priority = (last[0:paired:2], last[1:paired:2] + last[paired:])

  def start_static(first, end):
    for n in range(first, end):
      for priority in range(2):
        b, i = divmod(n + priority * _LAG, len(pairs))
        if 0 <= b < first_last:
          step, sub = divmod(b, _BATCHES)
          r, c, m = pairs[i]
          copy = copier(k_hbm if b < first_v else v_hbm, step)
          copy(m + priority, sub * burst_rows + r, _ROWS, c, half,
               None).start(priority=priority)
        elif b >= first_last:
          i += (b - first_last) * len(pairs)
          if i < len(last_by_priority[priority]):
            last_by_priority[priority][i][1].start(priority=priority)

  def start_burst(src, b):
    copies = [(copier(src, div(b + d, _BATCHES)),
               rem(b + d, _BATCHES) * burst_rows) for d in range(early + 1)]
    for n in range(len(pairs)):
      for priority in range(2):
        d, i = divmod(n + priority * _LAG, len(pairs))
        r, c, m = pairs[i]
        copy, row = copies[d]
        copy(m + priority, row + r, _ROWS, c, half,
             None).start(priority=priority)

  def score(step, batch):
    group, u, slot = locate(step)
    first = (group * _BATCHES + batch) * heads
    row = lax.broadcasted_iota(jnp.int32, (8, skv), 0)
    for j in range(_PARTS):
      h, part = div(j * heads + u, _PARTS), rem(j * heads + u, _PARTS)
      rows = pl.ds(pl.multiple_of(first + div(h, 8) * 8, 8), 8)
      s = jnp.dot(
          q_parts[part, rows, :].astype(buf.dtype),
          buf[slot, batch, pl.ds(pl.multiple_of(part * chunk, chunk), chunk), :],
          preferred_element_type=jnp.float32)
      s_ref[rows, :] += jnp.where(row == rem(h, 8), s, 0.0)

    @pl.when(u == heads - 1)
    def _():
      rows = pl.ds(pl.multiple_of(first, heads), heads)
      s = s_ref[rows, :] * scale
      p = jnp.exp(s - jnp.max(s, axis=-1, keepdims=True))
      p_ref[rows, :] = p.astype(p_ref.dtype)
      rl_ref[rows, :] = jnp.broadcast_to(
          1.0 / jnp.sum(p, axis=-1, keepdims=True), (heads, dh))

  def attend(step, batch, c=0, w=skv, done=None):
    group, u, slot = locate(step)
    rows = pl.ds(_aligned((group * _BATCHES + batch) * heads, heads), heads)
    o = lax.dot_general(
        p_ref[rows, pl.ds(c, w)], buf[slot, batch, :, pl.ds(c, w)],
        (((1,), (1,)), ((), ())), preferred_element_type=jnp.float32)
    h = lax.broadcasted_iota(jnp.int32, (heads, dh), 0)
    d = lax.broadcasted_iota(jnp.int32, (heads, dh), 1)
    part = sum((d >= j * chunk).astype(jnp.int32) for j in range(1, _PARTS))
    mine = ((_PARTS * h + part) & (heads - 1)) == u
    acc = acc_ref[rows, :] + jnp.where(mine, o, 0.0)
    acc_ref[rows, :] = acc

    @pl.when(u == heads - 1 if done is None else done)
    def _():
      o_ref[rows, :] = (acc * rl_ref[rows, :]).astype(o_ref.dtype)

  q_copy = pltpu.make_async_copy(q_hbm, q_ref, io_sem.at[0])

  def body(b, carry):
    pl.when(b < first_v - early)(lambda: start_burst(k_hbm, b))
    pl.when((b >= first_v) & (b < first_last - early))(
        lambda: start_burst(v_hbm, b))
    for x in (*range(first_v - early, first_v),
              *range(first_last - early, n_bursts)):
      pl.when(b == x)(functools.partial(
          start_static, x * len(pairs), (x + 1) * len(pairs)))

    @pl.when(b == 1)
    def _():
      q_copy.start()
      s_ref[...] = jnp.zeros_like(s_ref)
      acc_ref[...] = jnp.zeros_like(acc_ref)

    @pl.when(b == 2)
    def _():
      q_copy.wait()
      for j in range(_PARTS):
        q_parts[j] = q_ref[:, j * chunk:(j + 1) * chunk].astype(q_parts.dtype)

    @pl.when(b >= _WAIT_BURST)
    def _():
      since = jnp.maximum(b - _WAIT_BURST, 0)
      step, sub = div(since, _BATCHES), rem(since, _BATCHES)
      slot = locate(step)[2]
      pl.when(sub == 0)(pltpu.make_async_copy(
          buf.at[slot], buf.at[slot], step_sem.at[slot]).wait)

      @pl.when(sub < 2)
      def _():
        for consume, when in ((score, step < steps), (attend, step >= steps)):
          pl.when(when)(lambda: lax.fori_loop(
              0, _BATCHES // 2,
              lambda i, _: consume(step, sub * (_BATCHES // 2) + i), None))

    return carry

  n_bursts = first_last - _BATCHES + _WAIT_BURST + 2
  start_static(-_LAG, 0)
  lax.fori_loop(0, n_bursts, body, None)

  def o_copy(first, end):
    rows = pl.ds(first, end - first)
    return pltpu.make_async_copy(o_ref.at[rows], o_hbm.at[rows], io_sem.at[1])

  started = n_bursts * len(pairs)
  total = first_last * len(pairs) + len(last_by_priority[0])
  final = n_heads - (_BATCHES - _LAST_STEP[-1][0][0]) * heads
  for i, blocks in enumerate(_LAST_STEP):
    arrived = 1 + max(n for n, (j, _) in enumerate(last) if j == i) // 2
    upto = min(total, first_last * len(pairs) + arrived + _IN_FLIGHT)
    start_static(started, upto)
    started = max(started, upto)
    for j, copy in last:
      if j == i:
        copy.wait()
    if i == len(_LAST_STEP) - 1:
      o_copy(0, final).start()
    for batch, c, w in blocks:
      attend(2 * steps - 1, batch, c * skv // 8, w * skv // 8, done=c + w == 8)
  o_copy(final, n_heads).start()
  o_copy(0, n_heads).wait()


@jax.jit
def pallas_standalone__softmax_full_bidir__sampling_kernel(
    q: jax.Array,
    k: jax.Array,
    v: jax.Array,
):
  b, h, sq, dh = q.shape
  skv = k.shape[2]
  assert sq == 1 and b % _BATCHES == 0 and h % 8 == 0 and h & (h - 1) == 0
  assert dh % (_PARTS * _BATCHES * _ROWS) == 0 and skv % (8 * 128) == 0
  n = b * h
  hbm = pl.BlockSpec(memory_space=pl.ANY)
  out = pl.pallas_call(
      functools.partial(_kernel, heads=h, scale=dh**-0.5),
      in_specs=[hbm, hbm, hbm],
      out_specs=hbm,
      out_shape=jax.ShapeDtypeStruct((n, dh), q.dtype),
      scratch_shapes=[
          pltpu.VMEM((n, dh), q.dtype),
          pltpu.VMEM((_PARTS, n, dh // _PARTS), jnp.float32),
          pltpu.VMEM((_SLOTS, _BATCHES, dh, skv), k.dtype),
          pltpu.VMEM((n, skv), jnp.float32),
          pltpu.VMEM((n, skv), v.dtype),
          pltpu.VMEM((n, dh), jnp.float32),
          pltpu.VMEM((n, dh), jnp.float32),
          pltpu.VMEM((n, dh), q.dtype),
          pltpu.SemaphoreType.DMA((_SLOTS,)),
          pltpu.SemaphoreType.DMA((len(_LAST_STEP),)),
          pltpu.SemaphoreType.DMA((2,)),
      ],
      compiler_params=pltpu.CompilerParams(
          vmem_limit_bytes=64 * 1024 * 1024,
          disable_bounds_checks=True,
          disable_semaphore_checks=True,
      ),
  )(
      q.reshape(n, dh),
      jnp.swapaxes(k, 2, 3).reshape(n * dh, skv),
      jnp.swapaxes(v, 2, 3).reshape(n * dh, skv),
  )
  return out.reshape(b, h, sq, dh)
```

```python
import functools

import jax
import jax.numpy as jnp
from jax import lax
import jax.experimental.pallas as pl
import jax.experimental.pallas.tpu as pltpu

_PARTS = 3
_BATCHES = 4
_ROWS = 8
_LAG = 26
_IN_FLIGHT = 32
_SLOTS = 4
_WAIT_BURST = 5
_LAST_STEP = (
    ((0, 0, 4), (1, 0, 4)),
    ((2, 0, 4), (3, 0, 4)),
    ((0, 4, 4), (1, 4, 4)),
    ((2, 4, 4),),
    ((3, 4, 2),),
    ((3, 6, 1),),
    ((3, 7, 1),),
)


def _aligned(x, n):
  return x if isinstance(x, int) else pl.multiple_of(x, n)


def _kernel(q_hbm, k_hbm, v_hbm, o_hbm,
            q_ref, q_parts, buf, s_ref, p_ref, rl_ref, acc_ref, o_ref,
            step_sem, last_sem, io_sem, *, heads, scale):
  n_heads, dh = q_hbm.shape
  skv = k_hbm.shape[1]
  chunk = dh // _PARTS
  streams = _PARTS * _BATCHES
  groups = n_heads // (heads * _BATCHES)
  steps = groups * heads
  burst_rows = chunk // _BATCHES
  half = skv // 2
  pairs = [(r, c, m) for r in range(0, burst_rows, _ROWS) for c in (0, half)
           for m in range(0, streams, 2)]
  first_v = steps * _BATCHES
  first_last = (2 * steps - 1) * _BATCHES
  early = pl.cdiv(_LAG, len(pairs))

  def div(x, n):
    return x // n if isinstance(x, int) else lax.div(x, n)

  def rem(x, n):
    return x % n if isinstance(x, int) else lax.rem(x, n)

  def locate(step):
    return rem(div(step, heads), groups), rem(step, heads), rem(step, _SLOTS)

  def copier(src, step):
    group, u, slot = locate(step)
    base = (group * streams * heads + u) * chunk
    part = [rem(j * heads + u, _PARTS) * chunk for j in range(_PARTS)]

    def copy(m, r, rows, c, cols, sem=None):
      batch, j = divmod(m, _PARTS)
      return pltpu.make_async_copy(
          src.at[pl.ds(_aligned(base + m * heads * chunk + r, _ROWS), rows),
                 pl.ds(c, cols)],
          buf.at[slot, batch, pl.ds(_aligned(part[j] + r, _ROWS), rows),
                 pl.ds(c, cols)],
          step_sem.at[slot] if sem is None else sem)

    return copy

  last_copy = copier(v_hbm, 2 * steps - 1)
  last = []
  for i, blocks in enumerate(_LAST_STEP):
    pieces = []
    for batch, c, w in blocks:
      rows = min(chunk, 4 * _ROWS // w)
      pieces += [(r, _PARTS * batch + j, rows, c * skv // 8, w * skv // 8)
                 for r in range(0, chunk, rows) for j in range(_PARTS)]
    last += [(i, last_copy(m, r, rows, c, w, last_sem.at[i]))
             for r, m, rows, c, w in sorted(pieces)]
  paired = len(last) - _LAG
  last_by_priority = (last[0:paired:2], last[1:paired:2] + last[paired:])

  def start_static(first, end):
    for n in range(first, end):
      for priority in range(2):
        b, i = divmod(n + priority * _LAG, len(pairs))
        if 0 <= b < first_last:
          step, sub = divmod(b, _BATCHES)
          r, c, m = pairs[i]
          copy = copier(k_hbm if b < first_v else v_hbm, step)
          copy(m + priority, sub * burst_rows + r, _ROWS, c,
               half).start(priority=priority)
        elif b >= first_last:
          i += (b - first_last) * len(pairs)
          if i < len(last_by_priority[priority]):
            last_by_priority[priority][i][1].start(priority=priority)

  def start_burst(src, b):
    copies = [(copier(src, div(b + d, _BATCHES)),
               rem(b + d, _BATCHES) * burst_rows) for d in range(early + 1)]
    for n in range(len(pairs)):
      for priority in range(2):
        d, i = divmod(n + priority * _LAG, len(pairs))
        r, c, m = pairs[i]
        copy, row = copies[d]
        copy(m + priority, row + r, _ROWS, c, half).start(priority=priority)

  def score(step, batch):
    group, u, slot = locate(step)
    first = (group * _BATCHES + batch) * heads
    row = lax.broadcasted_iota(jnp.int32, (8, skv), 0)
    for j in range(_PARTS):
      h, part = div(j * heads + u, _PARTS), rem(j * heads + u, _PARTS)
      rows = pl.ds(pl.multiple_of(first + div(h, 8) * 8, 8), 8)
      s = jnp.dot(
          q_parts[part, rows, :].astype(buf.dtype),
          buf[slot, batch, pl.ds(pl.multiple_of(part * chunk, chunk), chunk), :],
          preferred_element_type=jnp.float32)
      s_ref[rows, :] += jnp.where(row == rem(h, 8), s, 0.0)

    @pl.when(u == heads - 1)
    def _():
      rows = pl.ds(pl.multiple_of(first, heads), heads)
      s = s_ref[rows, :] * scale
      p = jnp.exp(s - jnp.max(s, axis=-1, keepdims=True))
      p_ref[rows, :] = p.astype(p_ref.dtype)
      rl_ref[rows, :] = jnp.broadcast_to(
          1.0 / jnp.sum(p, axis=-1, keepdims=True), (heads, dh))

  def attend(step, batch, c=0, w=skv, done=None):
    group, u, slot = locate(step)
    rows = pl.ds(_aligned((group * _BATCHES + batch) * heads, heads), heads)
    o = lax.dot_general(
        p_ref[rows, pl.ds(c, w)], buf[slot, batch, :, pl.ds(c, w)],
        (((1,), (1,)), ((), ())), preferred_element_type=jnp.float32)
    h = lax.broadcasted_iota(jnp.int32, (heads, dh), 0)
    d = lax.broadcasted_iota(jnp.int32, (heads, dh), 1)
    part = sum((d >= j * chunk).astype(jnp.int32) for j in range(1, _PARTS))
    mine = ((_PARTS * h + part) & (heads - 1)) == u
    acc = acc_ref[rows, :] + jnp.where(mine, o, 0.0)
    acc_ref[rows, :] = acc

    @pl.when(u == heads - 1 if done is None else done)
    def _():
      o_ref[rows, :] = (acc * rl_ref[rows, :]).astype(o_ref.dtype)

  q_copy = pltpu.make_async_copy(q_hbm, q_ref, io_sem.at[0])

  def body(b, carry):
    pl.when(b < first_v - early)(lambda: start_burst(k_hbm, b))
    pl.when((b >= first_v) & (b < first_last - early))(
        lambda: start_burst(v_hbm, b))
    for x in (*range(first_v - early, first_v),
              *range(first_last - early, n_bursts)):
      pl.when(b == x)(functools.partial(
          start_static, x * len(pairs), (x + 1) * len(pairs)))

    @pl.when(b == 1)
    def _():
      q_copy.start()
      s_ref[...] = jnp.zeros_like(s_ref)
      acc_ref[...] = jnp.zeros_like(acc_ref)

    @pl.when(b == 2)
    def _():
      q_copy.wait()
      for j in range(_PARTS):
        q_parts[j] = q_ref[:, j * chunk:(j + 1) * chunk].astype(q_parts.dtype)

    @pl.when(b >= _WAIT_BURST)
    def _():
      since = jnp.maximum(b - _WAIT_BURST, 0)
      step, sub = div(since, _BATCHES), rem(since, _BATCHES)
      slot = locate(step)[2]
      pl.when(sub == 0)(pltpu.make_async_copy(
          buf.at[slot], buf.at[slot], step_sem.at[slot]).wait)

      @pl.when(sub < 2)
      def _():
        for consume, when in ((score, step < steps), (attend, step >= steps)):
          pl.when(when)(lambda: lax.fori_loop(
              0, _BATCHES // 2,
              lambda i, _: consume(step, sub * (_BATCHES // 2) + i), None))

    return carry

  n_bursts = first_last - _BATCHES + _WAIT_BURST + 2
  start_static(-_LAG, 0)
  lax.fori_loop(0, n_bursts, body, None)

  def o_copy(first, end):
    rows = pl.ds(first, end - first)
    return pltpu.make_async_copy(o_ref.at[rows], o_hbm.at[rows], io_sem.at[1])

  started = n_bursts * len(pairs)
  total = first_last * len(pairs) + len(last_by_priority[0])
  final = n_heads - (_BATCHES - _LAST_STEP[-1][0][0]) * heads
  for i, blocks in enumerate(_LAST_STEP):
    arrived = 1 + max(n for n, (j, _) in enumerate(last) if j == i) // 2
    upto = min(total, first_last * len(pairs) + arrived + _IN_FLIGHT)
    start_static(started, upto)
    started = max(started, upto)
    for j, copy in last:
      if j == i:
        copy.wait()
    if i == len(_LAST_STEP) - 1:
      o_copy(0, final).start()
    for batch, c, w in blocks:
      attend(2 * steps - 1, batch, c * skv // 8, w * skv // 8, done=c + w == 8)
  o_copy(final, n_heads).start()
  o_copy(0, final).wait()
  o_copy(final, n_heads).wait()


@jax.jit
def pallas_standalone__softmax_full_bidir__sampling_kernel(
    q: jax.Array,
    k: jax.Array,
    v: jax.Array,
):
  b, h, sq, dh = q.shape
  skv = k.shape[2]
  assert sq == 1 and b % _BATCHES == 0 and h % 8 == 0 and h & (h - 1) == 0
  assert dh % (_PARTS * _BATCHES * _ROWS) == 0 and skv % (8 * 128) == 0
  n = b * h
  hbm = pl.BlockSpec(memory_space=pl.ANY)
  out = pl.pallas_call(
      functools.partial(_kernel, heads=h, scale=dh**-0.5),
      in_specs=[hbm, hbm, hbm],
      out_specs=hbm,
      out_shape=jax.ShapeDtypeStruct((n, dh), q.dtype),
      scratch_shapes=[
          pltpu.VMEM((n, dh), q.dtype),
          pltpu.VMEM((_PARTS, n, dh // _PARTS), jnp.float32),
          pltpu.VMEM((_SLOTS, _BATCHES, dh, skv), k.dtype),
          pltpu.VMEM((n, skv), jnp.float32),
          pltpu.VMEM((n, skv), v.dtype),
          pltpu.VMEM((n, dh), jnp.float32),
          pltpu.VMEM((n, dh), jnp.float32),
          pltpu.VMEM((n, dh), q.dtype),
          pltpu.SemaphoreType.DMA((_SLOTS,)),
          pltpu.SemaphoreType.DMA((len(_LAST_STEP),)),
          pltpu.SemaphoreType.DMA((2,)),
      ],
      compiler_params=pltpu.CompilerParams(
          vmem_limit_bytes=64 * 1024 * 1024,
          disable_semaphore_checks=True,
      ),
  )(
      q.reshape(n, dh),
      jnp.swapaxes(k, 2, 3).reshape(n * dh, skv),
      jnp.swapaxes(v, 2, 3).reshape(n * dh, skv),
  )
  return out.reshape(b, h, sq, dh)
```
